```python
import os as _os
_os.environ.setdefault('JAX_PLATFORMS', 'cpu')
import jax
import jax.numpy as jnp

def _softmax(x, axis=-1):
    return jax.nn.softmax(x, axis=axis)

def _gelu(x):
    return jax.nn.gelu(x, approximate=True)

def _silu(x):
    return jax.nn.silu(x)

def _sigmoid(x):
    return jax.nn.sigmoid(x)

def _layernorm(x, axis=-1, eps=1e-05):
    m = jnp.mean(x, axis=axis, keepdims=True)
    v = jnp.var(x, axis=axis, keepdims=True)
    return (x - m) / jnp.sqrt(v + eps)

def _scatter_add(tgt, idx, src, axis=0):
    return tgt.at[idx].add(src)

def _segment_sum(src, seg, n):
    return jax.ops.segment_sum(src, seg, n)

class _Rng:

    def __init__(self, key):
        self._k = key

    def _next(self):
        self._k, sub = jax.random.split(self._k)
        return sub

    def normal(self, shape):
        return jax.random.normal(self._next(), shape, dtype=jnp.bfloat16)

    def randint(self, lo, hi, shape):
        return jax.random.randint(self._next(), shape, lo, hi, dtype=jnp.int32)

    def uniform(self, shape, lo=0.0, hi=1.0):
        return jax.random.uniform(self._next(), shape, jnp.bfloat16, lo, hi)

    def permutation(self, n):
        return jax.random.permutation(self._next(), n)
kernel_name = 'parallel_sum__memory_aug_recurrent_mem_tr__dense_activation_gelu__prompt'

def setup_inputs():
    _rng = _Rng(jax.random.key(int.from_bytes(__import__("os").urandom(4), "little")))
    _w = lambda a: (lambda t: t.astype(jnp.bfloat16) if jnp.issubdtype(t.dtype, jnp.floating) else t)(jnp.asarray(a))

    def _A_setup():
        B, S, Dm = (1, 2048, 1024)
        H, Dh = (32, 128)
        M, seg = (8, 32)
        seg = min(seg, S)
        S = S // seg * seg
        return {'x': _w((lambda *s: _rng.normal(s) * 0.05)(B, S, Dm)), 'mem0': _w((lambda *s: _rng.normal(s) * 0.2)(B, M, Dm)), 'Wq': _w((lambda *s: _rng.normal(s) * 0.8)(Dm, H, Dh) * Dm ** (-0.5)), 'Wk': _w((lambda *s: _rng.normal(s) * 0.8)(Dm, H, Dh) * Dm ** (-0.5)), 'Wv': _w((lambda *s: _rng.normal(s) * 0.2)(Dm, H, Dh) * Dm ** (-0.5)), 'Wo': _w((lambda *s: _rng.normal(s) * 0.2)(H, Dh, Dm) * (H * Dh) ** (-0.5)), 'seg_len': seg}
    _A_in = _A_setup()

    def _B_setup():
        B, S, D, F = (1, 2048, 1024, 3584)
        return {'x': _w((lambda *s: _rng.normal(s) * 0.05)(B, S, D)), 'w1': _w((lambda *s: _rng.normal(s) * 0.1)(D, F) * D ** (-0.5)), 'b1': _w((lambda *s: _rng.normal(s) * 0.1)(F) * 0.01), 'w2': _w((lambda *s: _rng.normal(s) * 0.1)(F, D) * F ** (-0.5)), 'b2': _w((lambda *s: _rng.normal(s) * 0.05)(D) * 0.01)}
    _B_in = _B_setup()
    return {'A_x': _A_in['x'], 'A_mem0': _A_in['mem0'], 'A_Wq': _A_in['Wq'], 'A_Wk': _A_in['Wk'], 'A_Wv': _A_in['Wv'], 'A_Wo': _A_in['Wo'], 'A_seg_len': _A_in['seg_len'], 'B_x': _B_in['x'], 'B_w1': _B_in['w1'], 'B_b1': _B_in['b1'], 'B_w2': _B_in['w2'], 'B_b2': _B_in['b2']}

def reference(A_x, A_mem0, A_Wq, A_Wk, A_Wv, A_Wo, A_seg_len, B_x, B_w1, B_b1, B_w2, B_b2):

    def _A_ref(x, mem0, Wq, Wk, Wv, Wo, seg_len):
        B, S, Dm = x.shape
        H, Dh = (Wq.shape[1], Wq.shape[2])
        M = mem0.shape[1]
        scale = Dh ** (-0.5)
        n_seg = S // seg_len
        L = M + seg_len
        idx = jnp.arange(L)
        mask = (idx[:, None] < M) | (idx[:, None] >= idx[None, :])
        mem = mem0
        outs = []
        for s in range(n_seg):
            xs = x[:, s * seg_len:(s + 1) * seg_len, :].copy()
            h = jnp.concatenate([mem, xs], axis=1)
            q = jnp.einsum('btd,dhe->bhte', h, Wq)
            k = jnp.einsum('btd,dhe->bhte', h, Wk)
            v = jnp.einsum('btd,dhe->bhte', h, Wv)
            scores = jnp.einsum('bhqe,bhke->bhqk', q, k) * scale
            scores = jnp.where(mask[None, None], scores, -1000000000.0)
            p = _softmax(scores, axis=-1)
            o = jnp.einsum('bhqk,bhke->bhqe', p, v)
            o = jnp.einsum('bhte,hed->btd', o, Wo)
            mem = o[:, :M, :].copy()
            outs.append(o[:, M:, :])
        return jnp.concatenate(outs, axis=1)

    def _B_ref(x, w1, b1, w2, b2):
        h = jnp.einsum('bsd,df->bsf', x, w1) + b1
        h = _gelu(h)
        return jnp.einsum('bsf,fd->bsd', h, w2) + b2
    x = A_x
    xn = _layernorm(x, axis=-1)
    return x + _A_ref(xn, A_mem0, A_Wq, A_Wk, A_Wv, A_Wo, A_seg_len) + _B_ref(xn, B_w1, B_b1, B_w2, B_b2)
```

```python
import functools
import math

import jax
import jax.numpy as jnp
import jax.experimental.pallas as pl
import jax.experimental.pallas.tpu as pltpu

_BF = jnp.bfloat16
_F32 = jnp.float32
_GRP = 16
_HEAD_ROWS = 24


def _dot(a, b):
    return jnp.dot(a, b, preferred_element_type=_F32)


def _dot_nt(a, b):
    return jax.lax.dot_general(a, b, (((1,), (1,)), ((), ())), preferred_element_type=_F32)


@functools.partial(jax.jit, static_argnames=("A_seg_len",))
def pallas_parallel_sum__memory_aug_recurrent_mem_tr__dense_activation_gelu__prompt_kernel(
    A_x: jax.Array,
    A_mem0: jax.Array,
    A_Wq: jax.Array,
    A_Wk: jax.Array,
    A_Wv: jax.Array,
    A_Wo: jax.Array,
    A_seg_len: int,
    B_x: jax.Array,
    B_w1: jax.Array,
    B_b1: jax.Array,
    B_w2: jax.Array,
    B_b2: jax.Array,
):
    del B_x
    B, S, D = A_x.shape
    _, MM, _ = A_mem0.shape
    _, H, E = A_Wq.shape
    F = B_w1.shape[1]
    SEG = int(A_seg_len)
    assert B == 1 and MM == 8 and SEG == 32 and E == 128, "kernel is specialised to these settings"
    assert S % (SEG * _GRP) == 0 and D % 128 == 0 and F % 128 == 0
    NS = S // SEG
    NG = NS // _GRP
    L = MM + SEG
    TAIL = SEG - _HEAD_ROWS
    MCH = MM + _HEAD_ROWS
    HE = H * E
    ND = D // 128
    NF = F // 128
    scale = float(E) ** -0.5
    DC = 128
    RC = 512

    def kernel(x_ref, mem0_ref, wq_hbm, wk_hbm, wv_hbm, wo_hbm, w1_hbm, b1_ref, w2_hbm, b2_ref,
               out_ref,
               sq, sk, sv, so, s1, s2,
               st3, sto, st2,
               xn, xt,
               qs, ks, vs,
               qt, kt, vt,
               mem, oall, otail, hbuf, ybuf,
               sem):
        def dma(src, dst):
            cp = pltpu.make_async_copy(src, dst, sem)
            cp.start()
            cp.wait()

        for w_hbm, s_ref in ((wq_hbm, sq), (wk_hbm, sk), (wv_hbm, sv)):
            for c in range(D // DC):
                dma(w_hbm.at[pl.ds(c * DC, DC)], st3)
                s_ref[:, pl.ds(c * DC, DC), :] = jnp.swapaxes(st3[...], 0, 1)
        for c in range(HE // RC):
            dma(wo_hbm.at[pl.ds(c * (RC // E), RC // E)], sto)
            for j in range(ND):
                so[j, pl.ds(c * RC, RC), :] = sto[:, :, pl.ds(128 * j, 128)].reshape(RC, 128)
        for c in range(D // RC):
            dma(w1_hbm.at[pl.ds(c * RC, RC)], st2)
            for j in range(NF):
                s1[j, pl.ds(c * RC, RC), :] = st2[:, pl.ds(128 * j, 128)]
        for c in range(F // RC):
            dma(w2_hbm.at[pl.ds(c * RC, RC)], st2.at[:, pl.ds(0, D)])
            for j in range(ND):
                s2[j, pl.ds(c * RC, RC), :] = st2[:, pl.ds(128 * j, 128)]

        LNR = 256
        def ln_body(b, carry):
            r0 = pl.multiple_of(b * LNR, LNR)
            xb = x_ref[0, pl.ds(r0, LNR), :].astype(_F32)
            mu = jnp.mean(xb, axis=-1, keepdims=True)
            xc = xb - mu
            var = jnp.mean(xc * xc, axis=-1, keepdims=True)
            xb = xc * jax.lax.rsqrt(var + 1e-5)
            xn[pl.ds(r0, LNR), :] = xb.astype(_BF)
            nseg = LNR // SEG
            tail = xb.reshape(nseg, SEG, D)[:, _HEAD_ROWS:, :].reshape(nseg * TAIL, D)
            xt[pl.ds(pl.multiple_of(b * (nseg * TAIL), nseg * TAIL), nseg * TAIL), :] = tail.astype(_BF)
            return carry
        jax.lax.fori_loop(0, S // LNR, ln_body, 0)

        mem[...] = mem0_ref[0].astype(_F32)

        def qkv_pass(lhs, slot_mem, slot_tok, write_mem):
            for w_ref, dst in ((sq, qs), (sk, ks), (sv, vs)):
                for h in range(H):
                    r = _dot(lhs, w_ref[h])
                    if write_mem:
                        dst[slot_mem, h, pl.ds(0, MM), :] = r[:MM]
                    dst[slot_tok, h, pl.ds(MM, _HEAD_ROWS), :] = r[MM:]

        def chain_lhs(tok_row0):
            tok = xn[pl.ds(tok_row0, _HEAD_ROWS), :].astype(_F32)
            return jnp.concatenate([mem[...], tok], axis=0).astype(_BF)

        qkv_pass(chain_lhs(0), 0, 0, write_mem=False)

        row = jax.lax.broadcasted_iota(jnp.int32, (L, L), 0)
        col = jax.lax.broadcasted_iota(jnp.int32, (L, L), 1)
        mask = (row < MM) | (row >= col)

        def step(s, carry):
            r = s % _GRP
            slot = s % 2
            nslot = 1 - slot

            @pl.when(r == 0)
            def _():
                g = s // _GRP
                nr = _GRP * TAIL
                lhs = xt[pl.ds(pl.multiple_of(g * nr, nr), nr), :]
                for w_ref, dst in ((sq, qt), (sk, kt), (sv, vt)):
                    for h in range(H):
                        dst[h] = _dot(lhs, w_ref[h])

            t0 = pl.multiple_of(r * TAIL, TAIL)
            for src, dst in ((qt, qs), (kt, ks), (vt, vs)):
                dst[slot, :, pl.ds(MCH, TAIL), :] = src[:, pl.ds(t0, TAIL), :]

            nxt = jnp.minimum(s + 1, NS - 1)
            qkv_pass(chain_lhs(pl.multiple_of(nxt * SEG, SEG)), slot, nslot, write_mem=True)

            for h in range(H):
                q = qs[slot, h].astype(_BF)
                k = ks[slot, h].astype(_BF)
                v = vs[slot, h].astype(_BF)
                sc = _dot_nt(q, k) * scale
                sc = jnp.where(mask, sc, -1e9)
                sc = sc - jnp.max(sc, axis=-1, keepdims=True)
                p = jnp.exp(sc)
                p = p / jnp.sum(p, axis=-1, keepdims=True)
                oall[:, pl.ds(h * E, E)] = _dot(p.astype(_BF), v)

            olhs = oall[pl.ds(0, MCH), :].astype(_BF)
            a_cols = [_dot(olhs, so[j]) for j in range(ND)]
            a_full = jnp.concatenate(a_cols, axis=1)
            mem[...] = a_full[:MM].astype(_BF).astype(_F32)
            otail[pl.ds(t0, TAIL), :] = oall[pl.ds(MCH, TAIL), :]

            x0 = pl.multiple_of(s * SEG, SEG)
            xs = xn[pl.ds(x0, SEG), :]
            for j in range(NF):
                hj = _dot(xs, s1[j]) + b1_ref[pl.ds(j * 128, 128)].astype(_F32)[None, :]
                hbuf[:, pl.ds(j * 128, 128)] = jax.nn.gelu(hj, approximate=True).astype(_BF)
            hb = hbuf[...]
            b_cols = [_dot(hb, s2[j]) for j in range(ND)]
            b_full = jnp.concatenate(b_cols, axis=1) + b2_ref[...].astype(_F32)[None, :]

            xres = x_ref[0, pl.ds(x0, SEG), :].astype(_F32) + b_full
            y0 = pl.multiple_of(r * SEG, SEG)
            ybuf[pl.ds(y0, _HEAD_ROWS), :] = xres[:_HEAD_ROWS] + a_full[MM:]
            ybuf[pl.ds(y0 + _HEAD_ROWS, TAIL), :] = xres[_HEAD_ROWS:]

            @pl.when(r == _GRP - 1)
            def _():
                g = s // _GRP
                tl = otail[...].astype(_BF)
                at = jnp.concatenate([_dot(tl, so[j]) for j in range(ND)], axis=1)
                for i in range(_GRP):
                    sl = pl.ds(i * SEG + _HEAD_ROWS, TAIL)
                    ybuf[sl, :] = ybuf[sl, :] + at[i * TAIL:(i + 1) * TAIL]
                nrow = _GRP * SEG
                out_ref[0, pl.ds(pl.multiple_of(g * nrow, nrow), nrow), :] = ybuf[...].astype(out_ref.dtype)

            return carry

        jax.lax.fori_loop(0, NS, step, 0)

    vm = pltpu.VMEM
    scratch = [
        vm((H, D, E), _BF), vm((H, D, E), _BF), vm((H, D, E), _BF),
        vm((ND, HE, 128), _BF), vm((NF, D, 128), _BF), vm((ND, F, 128), _BF),
        vm((DC, H, E), _BF), vm((RC // E, E, D), _BF), vm((RC, F), _BF),
        vm((S, D), _BF), vm((NS * TAIL, D), _BF),
        vm((2, H, L, E), _F32), vm((2, H, L, E), _F32), vm((2, H, L, E), _F32),
        vm((H, _GRP * TAIL, E), _F32), vm((H, _GRP * TAIL, E), _F32), vm((H, _GRP * TAIL, E), _F32),
        vm((MM, D), _F32), vm((L, HE), _F32), vm((_GRP * TAIL, HE), _F32),
        vm((SEG, F), _BF), vm((_GRP * SEG, D), _F32),
        pltpu.SemaphoreType.DMA(()),
    ]
    any_spec = pl.BlockSpec(memory_space=pl.ANY)
    return pl.pallas_call(
        kernel,
        in_specs=[pl.BlockSpec(), pl.BlockSpec(),
                  any_spec, any_spec, any_spec, any_spec, any_spec,
                  pl.BlockSpec(), any_spec, pl.BlockSpec()],
        out_specs=pl.BlockSpec(),
        out_shape=jax.ShapeDtypeStruct(A_x.shape, A_x.dtype),
        scratch_shapes=scratch,
        compiler_params=pltpu.CompilerParams(vmem_limit_bytes=110 * 1024 * 1024),
    )(A_x, A_mem0, A_Wq, A_Wk, A_Wv, A_Wo, B_w1, B_b1, B_w2, B_b2)
```

```python
import functools
import math

import jax
import jax.numpy as jnp
import jax.experimental.pallas as pl
import jax.experimental.pallas.tpu as pltpu

_BF = jnp.bfloat16
_F32 = jnp.float32
_GRP = 16
_HEAD_ROWS = 24


def _dot(a, b):
    return jnp.dot(a, b, preferred_element_type=_F32)


def _dot_nt(a, b):
    return jax.lax.dot_general(a, b, (((1,), (1,)), ((), ())), preferred_element_type=_F32)


@functools.partial(jax.jit, static_argnames=("A_seg_len",))
def pallas_parallel_sum__memory_aug_recurrent_mem_tr__dense_activation_gelu__prompt_kernel(
    A_x: jax.Array,
    A_mem0: jax.Array,
    A_Wq: jax.Array,
    A_Wk: jax.Array,
    A_Wv: jax.Array,
    A_Wo: jax.Array,
    A_seg_len: int,
    B_x: jax.Array,
    B_w1: jax.Array,
    B_b1: jax.Array,
    B_w2: jax.Array,
    B_b2: jax.Array,
):
    del B_x
    B, S, D = A_x.shape
    _, MM, _ = A_mem0.shape
    _, H, E = A_Wq.shape
    F = B_w1.shape[1]
    SEG = int(A_seg_len)
    assert B == 1 and MM == 8 and SEG == 32 and E == 128, "kernel is specialised to these settings"
    assert S % (SEG * _GRP) == 0 and D % 128 == 0 and F % 128 == 0
    NS = S // SEG
    NG = NS // _GRP
    L = MM + SEG
    TAIL = SEG - _HEAD_ROWS
    MCH = MM + _HEAD_ROWS
    HE = H * E
    ND = D // 128
    NF = F // 128
    scale = float(E) ** -0.5
    DC = 128

    def kernel(x_ref, mem0_ref, wq_hbm, wk_hbm, wv_hbm, wo_hbm, w1_hbm, b1_ref, w2_hbm, b2_ref,
               out_ref,
               sq, sk, sv, so, s1, s2,
               st3,
               xn, xt,
               qs, ks, vs,
               qt, kt, vt,
               mem, oall, otail, hbuf, ybuf, obuf,
               sems):
        sq32, sk32, sv32 = (r.bitcast(jnp.uint32) for r in (sq, sk, sv))
        so32, s132, s232 = (r.bitcast(jnp.uint32) for r in (so, s1, s2))

        def wslab(ref32, i):
            w = ref32[i]
            return pltpu.bitcast(w.reshape(-1, w.shape[-1]), _BF)

        NCH = D // DC
        nchunks = 3 * NCH

        def chunk_copy(i):
            w_hbm = (wq_hbm, wk_hbm, wv_hbm)[i // NCH]
            return pltpu.make_async_copy(w_hbm.at[pl.ds((i % NCH) * DC, DC)], st3.at[i % 2], sems.at[i % 2])

        def slab_copies():
            cps = []
            for j in range(ND):
                cps.append(pltpu.make_async_copy(wo_hbm.at[:, :, pl.ds(128 * j, 128)], so.at[j], sems.at[2 + j]))
            for j in range(NF):
                cps.append(pltpu.make_async_copy(w1_hbm.at[:, pl.ds(128 * j, 128)], s1.at[j], sems.at[2 + ND + j]))
            for j in range(ND):
                cps.append(pltpu.make_async_copy(w2_hbm.at[:, pl.ds(128 * j, 128)], s2.at[j], sems.at[2 + ND + NF + j]))
            return cps

        chunk_copy(0).start()
        chunk_copy(1).start()
        for i in range(nchunks):
            chunk_copy(i).wait()
            dst = (sq, sk, sv)[i // NCH]
            dst[:, pl.ds((i % NCH) * DC, DC), :] = jnp.swapaxes(st3[i % 2], 0, 1)
            if i + 2 < nchunks:
                chunk_copy(i + 2).start()
            if i + 3 == nchunks:
                for cp in slab_copies():
                    cp.start()

        LNR = 256
        def ln_body(b, carry):
            r0 = pl.multiple_of(b * LNR, LNR)
            xb = x_ref[0, pl.ds(r0, LNR), :].astype(_F32)
            mu = jnp.mean(xb, axis=-1, keepdims=True)
            xc = xb - mu
            var = jnp.mean(xc * xc, axis=-1, keepdims=True)
            xb = xc * jax.lax.rsqrt(var + 1e-5)
            xn[pl.ds(r0, LNR), :] = xb.astype(_BF)
            nseg = LNR // SEG
            tail = xb.reshape(nseg, SEG, D)[:, _HEAD_ROWS:, :].reshape(nseg * TAIL, D)
            xt[pl.ds(pl.multiple_of(b * (nseg * TAIL), nseg * TAIL), nseg * TAIL), :] = tail.astype(_BF)
            return carry
        jax.lax.fori_loop(0, S // LNR, ln_body, 0)

        mem[...] = mem0_ref[0].astype(_F32)

        def qkv_pass(lhs, slot_mem, slot_tok, write_mem):
            for w_ref, dst in ((sq32, qs), (sk32, ks), (sv32, vs)):
                for h in range(H):
                    r = _dot(lhs, wslab(w_ref, h))
                    if write_mem:
                        dst[slot_mem, h, pl.ds(0, MM), :] = r[:MM]
                    dst[slot_tok, h, pl.ds(MM, _HEAD_ROWS), :] = r[MM:]

        def chain_lhs(tok_row0):
            tok = xn[pl.ds(tok_row0, _HEAD_ROWS), :].astype(_F32)
            return jnp.concatenate([mem[...], tok], axis=0).astype(_BF)

        def bulk_qkv(g):
            nr = _GRP * TAIL
            lhs = xt[pl.ds(pl.multiple_of(g * nr, nr), nr), :]
            for w_ref, dst in ((sq32, qt), (sk32, kt), (sv32, vt)):
                for h in range(H):
                    dst[h] = _dot(lhs, wslab(w_ref, h))

        qkv_pass(chain_lhs(0), 0, 0, write_mem=False)
        bulk_qkv(0)
        for cp in slab_copies():
            cp.wait()

        row = jax.lax.broadcasted_iota(jnp.int32, (L, L), 0)
        col = jax.lax.broadcasted_iota(jnp.int32, (L, L), 1)
        mask = (row < MM) | (row >= col)

        def step(s, carry):
            r = s % _GRP
            slot = s % 2
            nslot = 1 - slot

            @pl.when(jnp.logical_and(r == 0, s > 0))
            def _():
                bulk_qkv(s // _GRP)

            t0 = pl.multiple_of(r * TAIL, TAIL)
            for src, dst in ((qt, qs), (kt, ks), (vt, vs)):
                dst[slot, :, pl.ds(MCH, TAIL), :] = src[:, pl.ds(t0, TAIL), :]

            nxt = jnp.minimum(s + 1, NS - 1)
            qkv_pass(chain_lhs(pl.multiple_of(nxt * SEG, SEG)), slot, nslot, write_mem=True)

            x0 = pl.multiple_of(s * SEG, SEG)
            xs = xn[pl.ds(x0, SEG), :]
            for h in range(H):
                if h % 4 == 0:
                    for j in range(h, min(h + 4, NF)):
                        hj = _dot(xs, wslab(s132, j)) + b1_ref[pl.ds(j * 128, 128)].astype(_F32)[None, :]
                        hbuf[:, pl.ds(j * 128, 128)] = jax.nn.gelu(hj, approximate=True).astype(_BF)
                q = qs[slot, h].astype(_BF)
                k = ks[slot, h].astype(_BF)
                v = vs[slot, h].astype(_BF)
                sc = _dot_nt(q, k) * scale
                sc = jnp.where(mask, sc, -1e9)
                sc = sc - jnp.max(sc, axis=-1, keepdims=True)
                p = jnp.exp(sc)
                p = p / jnp.sum(p, axis=-1, keepdims=True)
                oall[:, pl.ds(h * E, E)] = _dot(p.astype(_BF), v)

            olhs = oall[pl.ds(0, MCH), :].astype(_BF)
            a_cols = [_dot(olhs, wslab(so32, j)) for j in range(ND)]
            a_full = jnp.concatenate(a_cols, axis=1)
            mem[...] = a_full[:MM].astype(_BF).astype(_F32)
            otail[pl.ds(t0, TAIL), :] = oall[pl.ds(MCH, TAIL), :]

            hb = hbuf[...]
            b_cols = [_dot(hb, wslab(s232, j)) for j in range(ND)]
            b_full = jnp.concatenate(b_cols, axis=1) + b2_ref[...].astype(_F32)[None, :]

            xres = x_ref[0, pl.ds(x0, SEG), :].astype(_F32) + b_full
            y0 = pl.multiple_of(r * SEG, SEG)
            ybuf[pl.ds(y0, _HEAD_ROWS), :] = xres[:_HEAD_ROWS] + a_full[MM:]
            ybuf[pl.ds(y0 + _HEAD_ROWS, TAIL), :] = xres[_HEAD_ROWS:]

            @pl.when(r == _GRP - 1)
            def _():
                g = s // _GRP
                tl = otail[...].astype(_BF)
                at = jnp.concatenate([_dot(tl, wslab(so32, j)) for j in range(ND)], axis=1)
                for i in range(_GRP):
                    sl = pl.ds(i * SEG + _HEAD_ROWS, TAIL)
                    ybuf[sl, :] = ybuf[sl, :] + at[i * TAIL:(i + 1) * TAIL]
                @pl.when(g > 0)
                def _():
                    out_copy(g - 1).wait()
                obuf[...] = ybuf[...].astype(obuf.dtype)
                out_copy(g).start()

            return carry

        def out_copy(g):
            nrow = _GRP * SEG
            return pltpu.make_async_copy(obuf, out_ref.at[0, pl.ds(pl.multiple_of(g * nrow, nrow), nrow), :],
                                         sems.at[2 + ND + NF + ND])

        jax.lax.fori_loop(0, NS, step, 0)
        out_copy(NG - 1).wait()

    vm = pltpu.VMEM
    scratch = [
        vm((H, D, E), _BF), vm((H, D, E), _BF), vm((H, D, E), _BF),
        vm((ND, H, E, 128), _BF), vm((NF, D, 128), _BF), vm((ND, F, 128), _BF),
        vm((2, DC, H, E), _BF),
        vm((S, D), _BF), vm((NS * TAIL, D), _BF),
        vm((2, H, L, E), _F32), vm((2, H, L, E), _F32), vm((2, H, L, E), _F32),
        vm((H, _GRP * TAIL, E), _F32), vm((H, _GRP * TAIL, E), _F32), vm((H, _GRP * TAIL, E), _F32),
        vm((MM, D), _F32), vm((L, HE), _F32), vm((_GRP * TAIL, HE), _F32),
        vm((SEG, F), _BF), vm((_GRP * SEG, D), _F32), vm((_GRP * SEG, D), _BF),
        pltpu.SemaphoreType.DMA((2 + ND + NF + ND + 1,)),
    ]
    any_spec = pl.BlockSpec(memory_space=pl.ANY)
    return pl.pallas_call(
        kernel,
        in_specs=[pl.BlockSpec(), pl.BlockSpec(),
                  any_spec, any_spec, any_spec, any_spec, any_spec,
                  pl.BlockSpec(), any_spec, pl.BlockSpec()],
        out_specs=any_spec,
        out_shape=jax.ShapeDtypeStruct(A_x.shape, A_x.dtype),
        scratch_shapes=scratch,
        compiler_params=pltpu.CompilerParams(vmem_limit_bytes=110 * 1024 * 1024),
    )(A_x, A_mem0, A_Wq, A_Wk, A_Wv, A_Wo, B_w1, B_b1, B_w2, B_b2)
```
